```python
import os as _os
_os.environ.setdefault("JAX_PLATFORMS", "cpu")
import jax
import jax.numpy as jnp

def _softmax(x, axis=-1):
    return jax.nn.softmax(x, axis=axis)
def _gelu(x):
    return jax.nn.gelu(x, approximate=True)
def _silu(x):
    return jax.nn.silu(x)
def _sigmoid(x):
    return jax.nn.sigmoid(x)
def _layernorm(x, axis=-1, eps=1e-5):
    m = jnp.mean(x, axis=axis, keepdims=True)
    v = jnp.var(x, axis=axis, keepdims=True)
    return (x - m) / jnp.sqrt(v + eps)
def _scatter_add(tgt, idx, src, axis=0):
    return tgt.at[idx].add(src)
def _segment_sum(src, seg, n):
    return jax.ops.segment_sum(src, seg, n)
class _Rng:
    def __init__(self, key):
        self._k = key
    def _next(self):
        self._k, sub = jax.random.split(self._k)
        return sub
    def normal(self, shape):
        return jax.random.normal(self._next(), shape, dtype=jnp.bfloat16)
    def randint(self, lo, hi, shape):
        return jax.random.randint(self._next(), shape, lo, hi, dtype=jnp.int32)
    def uniform(self, shape, lo=0.0, hi=1.0):
        return jax.random.uniform(self._next(), shape, jnp.bfloat16, lo, hi)
    def permutation(self, n):
        return jax.random.permutation(self._next(), n)


kernel_name = 'sequential_preLN__sliding_block__dense_activation_gelu__prompt'

def setup_inputs():
    _rng = _Rng(jax.random.key(int.from_bytes(__import__("os").urandom(4), "little")))
    _w = (lambda a: (lambda t: t.astype(jnp.bfloat16) if jnp.issubdtype(t.dtype, jnp.floating) else t)(jnp.asarray(a)))
    def _A_setup():
        B, S, D = 1, 2048, 640
        return {
            "x": _w((lambda *s: _rng.normal(s) * 0.05)(B, S, D)),
            "wqkv": _w((lambda *s: _rng.normal(s) * 0.05)(D, 3 * D)),
            "wo": _w((lambda *s: _rng.normal(s) * 0.05)(D, D)),
        }
    _A_in = _A_setup()

    def _B_setup():
        B, S, D, F = 1, 2048, 640, 1536
        return {
            "x": _w((lambda *s: _rng.normal(s) * 0.05)(B, S, D)),
            "w1": _w((lambda *s: _rng.normal(s) * 0.8)(D, F) * (D ** -0.5)),
            "b1": _w((lambda *s: _rng.normal(s) * 0.8)(F) * 0.01),
            "w2": _w((lambda *s: _rng.normal(s) * 0.8)(F, D) * (F ** -0.5)),
            "b2": _w((lambda *s: _rng.normal(s) * 0.05)(D) * 0.01),
        }
    _B_in = _B_setup()

    return {
        "A_x": _A_in["x"],
        "A_wqkv": _A_in["wqkv"],
        "A_wo": _A_in["wo"],
        "B_x": _B_in["x"],
        "B_w1": _B_in["w1"],
        "B_b1": _B_in["b1"],
        "B_w2": _B_in["w2"],
        "B_b2": _B_in["b2"],
    }

def reference(A_x, A_wqkv, A_wo, B_x, B_w1, B_b1, B_w2, B_b2):
    def _A_ref(x, wqkv, wo):
        B, S, D = x.shape
        H = 32; Dh = D // H; W = 256
        qkv = (lambda x, *d: x.transpose(*d))((x @ wqkv).reshape(B, S, 3, H, Dh), 2, 0, 3, 1, 4)
        q, k, v = qkv[0], qkv[1], qkv[2]
        scores = jnp.einsum("bhqd,bhkd->bhqk", q, k) * (Dh ** -0.5)
        idx = jnp.arange(S)
        mask = (idx[:, None] - idx[None, :] >= 0) & (idx[:, None] - idx[None, :] < W)
        scores = jnp.where(mask[None, None], scores, -1e9)
        p = _softmax(scores, axis=-1)
        o = jnp.einsum("bhqk,bhkd->bhqd", p, v)
        return (lambda x, *d: x.transpose(*d))(o, 0, 2, 1, 3).reshape(B, S, D) @ wo

    def _B_ref(x, w1, b1, w2, b2):
        h = jnp.einsum("bsd,df->bsf", x, w1) + b1
        h = _gelu(h)
        return jnp.einsum("bsf,fd->bsd", h, w2) + b2

    x = A_x
    h = x + _A_ref(_layernorm(x, axis=-1), A_wqkv, A_wo)
    h2 = h + _B_ref(_layernorm(h, axis=-1), B_w1, B_b1, B_w2, B_b2)
    return h2
```

```python
import functools
import numpy as np
import jax
import jax.numpy as jnp
from jax.experimental import pallas as pl
from jax.experimental.pallas import tpu as pltpu

S, D, H, DH, W, F = 2048, 640, 32, 20, 256, 1536
NT = (((1,), (1,)), ((), ()))
QSCALE = float(DH ** -0.5 * np.log2(np.e))
NEG = -1e30
f32, bf16, u32 = jnp.float32, jnp.bfloat16, jnp.uint32

def _ln(x):
    m = jnp.mean(x, axis=-1, keepdims=True)
    xc = x - m
    v = jnp.mean(xc * xc, axis=-1, keepdims=True)
    return xc * jax.lax.rsqrt(v + 1e-5)

def _gelu(h):
    c = float(np.sqrt(2 / np.pi))
    t = jnp.tanh(h * (c + (c * 0.044715) * (h * h)))
    hh = 0.5 * h
    return hh + hh * t

GT = [(0, None), (0, 1), (1, None), (1, 2), (2, 3), (3, None), (3, 4), (4, None)]

def _mm(a, w_ref, c0, c1):
    kt, ntile = a.shape[1] // 128, (c1 - c0) // 128
    nfull = ntile
    while (nfull * kt) % 4:
        nfull -= 1
    cm = c0 + 128 * nfull
    outs = [jnp.dot(a, w_ref[:, c0:cm], preferred_element_type=f32)] if nfull else []
    if cm < c1:
        q = a.shape[0] // 4
        outs.append(jnp.concatenate([jnp.dot(a[q * i:q * (i + 1)], w_ref[:, cm:c1], preferred_element_type=f32)
                                     for i in range(4)], axis=0))
    return outs[0] if len(outs) == 1 else jnp.concatenate(outs, axis=1)

def make(BM=256, WO_AT=2, LC=32, W2_AT=2, TIE=(None, 0, 16, 32), FL={}):
    NB = BM // 128
    NS = S // BM
    def kern(x_hbm, wqkv_hbm, wo_hbm, w1_hbm, b1_hbm, w2_hbm, b2_hbm, o_ref, b1_ref, b2_ref,
             x_scr, wqkv_ref, wo_ref, w1_ref, w2_ref, xn_scr, k_scr, vt_scr, p_scr, s_scr, h_scr, sems):
        step = pl.program_id(0)
        cp_x0 = pltpu.make_async_copy(x_hbm.at[0:BM], x_scr.at[0:BM], sems.at[0])
        cp_w = [pltpu.make_async_copy(wqkv_hbm.at[:, D * j:D * (j + 1)], wqkv_ref.at[:, D * j:D * (j + 1)], sems.at[1 + j])
                for j in range(3)]
        cp_wo = pltpu.make_async_copy(wo_hbm, wo_ref, sems.at[4])
        cp_x1 = pltpu.make_async_copy(x_hbm.at[BM:2 * BM], x_scr.at[BM:2 * BM], sems.at[5])
        cp_x2 = pltpu.make_async_copy(x_hbm.at[2 * BM:S], x_scr.at[2 * BM:S], sems.at[8])
        cp_b1 = pltpu.make_async_copy(b1_hbm, b1_ref, sems.at[9])
        cp_b2 = pltpu.make_async_copy(b2_hbm, b2_ref, sems.at[10])
        cp_w1 = pltpu.make_async_copy(w1_hbm, w1_ref, sems.at[6])
        cp_w2 = pltpu.make_async_copy(w2_hbm, w2_ref, sems.at[7])

        def body(first):
            lane = jax.lax.broadcasted_iota(jnp.int32, (1, 128), 1)
            row0 = 0 if first else pl.multiple_of(step * BM, BM)
            blk0 = 0 if first else step * NB
            if first:
                cp_x0.start(); cp_w[0].start()
                cp_x0.wait()
                cp_w[1].start()
                xn = _ln(x_scr[0:BM].astype(f32)).astype(bf16)
                parts = []
                for j in range(3):
                    cp_w[j].wait()
                    for cp in ([cp_w[2]], [cp_wo, cp_b1, cp_b2], [cp_w1, cp_x1])[j]:
                        cp.start()
                    parts.append(_mm(xn, wqkv_ref, D * j, D * (j + 1)))
                qq, kq, vq = parts
            else:
                qkv = _mm(xn_scr[...], wqkv_ref, 0, 3 * D)
                qq, kq, vq = qkv[:, 0:D], qkv[:, D:2 * D], qkv[:, 2 * D:]
            qt = [qq[:, 128 * t:128 * (t + 1)] * QSCALE for t in range(5)]
            kt = [kq[:, 128 * t:128 * (t + 1)] for t in range(5)]
            grp = lambda ts, g: ts[GT[g][0]] if GT[g][1] is None else jnp.where(lane >= 64, ts[GT[g][0]], ts[GT[g][1]])
            for g in range(8):
                k_scr[g, pl.ds(row0, BM), :] = grp(kt, g).astype(bf16)
            def pack16(v):
                n = v.shape[0] // 16
                lo = jnp.concatenate([v[16 * m:16 * m + 8] for m in range(n)], axis=0)
                hi = jnp.concatenate([v[16 * m + 8:16 * m + 16] for m in range(n)], axis=0)
                return pltpu.pack_elementwise([lo, hi], packed_dtype=bf16)
            for b in range(NB):
                vp = pltpu.bitcast(pack16(vq[128 * b:128 * (b + 1)]), bf16).astype(f32)
                vt_scr[blk0 + b] = vp.T.astype(bf16)
            r = jax.lax.broadcasted_iota(jnp.int32, (64, 256), 0)
            c = jax.lax.broadcasted_iota(jnp.int32, (64, 256), 1)
            tri = r <= (c & 63)
            lo_half = (jax.lax.broadcasted_iota(jnp.int32, (1, 256), 1) & 64) == 0
            r2 = jax.lax.broadcasted_iota(jnp.int32, (64, 128), 0)
            c2 = jax.lax.broadcasted_iota(jnp.int32, (64, 128), 1)
            klo = r2 + (r2 & 56)
            pmask = [jnp.where(klo <= cq, jnp.uint32(0xFFFF), jnp.uint32(0)) | jnp.where(klo + 8 <= cq, jnp.uint32(0xFFFF0000), jnp.uint32(0))
                     for cq in (c2, c2 ^ 64)]
            zero_of = lambda t: jnp.minimum(jnp.maximum(t, 0.0), 0.0)
            sub = jax.lax.broadcasted_iota(jnp.int32, (8, 128), 0)
            sub16 = jax.lax.broadcasted_iota(jnp.int32, (16, 128), 0)
            ones_w = jnp.uint32(0x3F803F80)
            nt = lambda b: 3

            def qmask(b, g):
                qs = []
                for h in range(4 * g, 4 * g + 4):
                    lo, hi = DH * h, DH * h + DH
                    t0, t1 = lo // 128, (hi - 1) // 128
                    sl = slice(128 * b, 128 * (b + 1))
                    if t0 == t1:
                        qs.append(jnp.where((lane >= lo - 128 * t0) & (lane < hi - 128 * t0), qt[t0][sl], 0.0))
                    else:
                        qs.append(jnp.where(lane >= lo - 128 * t0, qt[t0][sl],
                                            jnp.where(lane < hi - 128 * t1, qt[t1][sl], 0.0)))
                return qs

            def qk_head(g):
                tri1 = (jax.lax.broadcasted_iota(jnp.int32, (128, 512), 0)
                        <= (jax.lax.broadcasted_iota(jnp.int32, (128, 512), 1) & 127))
                s0 = jax.lax.dot_general(k_scr[g, 0:128, :], jnp.concatenate(qmask(0, g), axis=0).astype(bf16), NT,
                                         preferred_element_type=f32)
                s1 = jax.lax.dot_general(k_scr[g, 0:256, :], jnp.concatenate(qmask(1, g), axis=0).astype(bf16), NT,
                                         preferred_element_type=f32)
                s0 = jnp.where(tri1, s0, NEG)
                s1 = jnp.concatenate([s1[0:128], jnp.where(tri1, s1[128:256], NEG)], axis=0)
                s_scr[g % 2, 0:128, :] = s0
                s_scr[g % 2, 128:384, :] = s1
                m0, m1 = jnp.max(s0, axis=0, keepdims=True), jnp.max(s1, axis=0, keepdims=True)
                tie = lambda s, t: s[t:t + 8, 384:512]
                return [m0, m1, m1], [None, tie(s0, 0), tie(s0, 96)]

            def qk(b, g):
                if first and b == 0:
                    return qk_head(g)
                qs = qmask(b, g)
                qe = jnp.concatenate([q[0:64] for q in qs], axis=0).astype(bf16)
                qo = jnp.concatenate([qs[i][64:128] for i in (1, 0, 3, 2)], axis=0).astype(bf16)
                n = nt(b)
                st = row0 + 128 * (b + 1 - n)
                kw = pltpu.bitcast(k_scr[g, pl.ds(st if first else pl.multiple_of(st, 128), 128 * n), :], u32)
                o0 = (3 - n) * 128
                kr = lambda R, sz: kw[(R - o0) // 2:(R - o0 + sz) // 2]
                ev = (0, 256, 64) if n == 3 else (256,)
                od = (256, 64, 320) if n == 3 else (256, 320)
                def run(offs, qq_):
                    ch = [kr(o + 16 * j, 16) for j in range(4) for o in offs]
                    if n > 1:
                        ch.append(kr(128, 128))
                    s = jax.lax.dot_general(pltpu.bitcast(jnp.concatenate(ch, axis=0), bf16), qq_, NT,
                                            preferred_element_type=f32)
                    L = len(offs)
                    d = {o: jnp.concatenate([s[16 * (L * j + i):16 * (L * j + i + 1)] for j in range(4)], axis=0)
                         for i, o in enumerate(offs)}
                    d[128] = s[64 * L:] if n > 1 else None
                    return d
                se, so = run(ev, qe), run(od, qo)
                xe = [jnp.where(tri, se[256], se.get(0, NEG)), se.get(64, jnp.full((64, 256), NEG, f32))]
                xo = [so[256], jnp.where(tri, so[320], so.get(64, NEG))]
                if n > 1:
                    xe.append(se[128]); xo.append(so[128])
                xe = jnp.concatenate(xe, axis=0); xo = jnp.concatenate(xo, axis=0)
                s = jnp.concatenate([jnp.where(lo_half, xe, xo), jnp.where(lo_half, xo, xe)], axis=1)
                s_scr[g % 2, 0:256, :] = s
                return [jnp.max(s, axis=0, keepdims=True)] * len(TIE), [None if t is None else s[t:t + 8, 384:512] for t in TIE]

            def sm_pv(b, g, s, ties):
                head = first and b == 0
                ms, _ = s
                cs = (384 if head else 256) // len(ms)
                for j, m in enumerate(ms):
                    m = jnp.broadcast_to(m, (8, 512))
                    if ties is not None and j < len(ties) and ties[j] is not None:
                        m = m + jnp.concatenate([zero_of(ties[j])] * 4, axis=1)
                    m = jnp.concatenate([m] * (cs // 8), axis=0)
                    p_scr[g % 2, cs * j // 2:cs * (j + 1) // 2, :] = pack16(jnp.exp2(s_scr[g % 2, cs * j:cs * (j + 1), :] - m))
                if head:
                    pv(0, g); pv(1, g)
                else:
                    pv(b, g)

            def pv(b, g):
                head = first and b < 2
                slot = g % 2
                rows = allrows[b]
                n = b + 1 if head else 3
                for i4, h in enumerate(range(4 * g, 4 * g + 4)):
                    col = 128 * (i4 if head else (0, 2, 1, 3)[i4])
                    if head:
                        ps = [p_scr[slot, 64 * b:64 * (2 * b + 1), col:col + 128]]
                    else:
                        pm = p_scr[slot, 0:64, col:col + 128]
                        p2 = pm & pmask[i4 % 2]
                        ps = [pm ^ p2, p2, p_scr[slot, 64:128, col:col + 128]]
                    a = (DH * h) // 16
                    off = DH * h - 16 * a
                    vs = []
                    for j in ((0,), (0, 1), (0, 2, 1))[n - 1]:
                        vw = pltpu.bitcast(vt_scr[blk0 + b + 1 - n + j, 16 * a:16 * a + 32, :], u32)
                        vs.append(jnp.where((sub16 >= 12) if off < 8 else (sub16 < 4), ones_w, vw))
                    o = jnp.dot(pltpu.bitcast(jnp.concatenate(vs, axis=1), bf16),
                                pltpu.bitcast(jnp.concatenate(ps, axis=0), bf16), preferred_element_type=f32)
                    if off < 8:
                        l, oo = o[24:32], o[0:24]
                    else:
                        l, oo = o[0:8], o[8:32]
                    rl = 1.0 / l
                    g0 = (DH * h) // 8
                    for i in range(3):
                        val = oo[8 * i:8 * (i + 1)] * rl
                        if i4 % 2 and not head:
                            val = pltpu.roll(val, 64, axis=1)
                        rows[g0 + i] = val if rows[g0 + i] is None else jnp.where(sub < 4, rows[g0 + i], val)

            allrows = [[None] * 80 for _ in range(NB)]
            hn, gl = {b: [] for b in range(NB)}, {}
            rep = lambda z, n: jnp.concatenate([jnp.concatenate([z] * 5, axis=1)] * (n // 8), axis=0)
            def wo(b):
                att = jnp.concatenate(allrows[b], axis=0).T.astype(bf16)
                st = row0 + 128 * b
                xx = x_scr[pl.ds(st if first else pl.multiple_of(st, 128), 128), :].astype(f32)
                h_scr[128 * b:128 * (b + 1), :] = xx + _mm(att, wo_ref, 0, D)
            def ln2(b, tie=None):
                r0 = 128 * b + LC * len(hn[b])
                v = h_scr[r0:r0 + LC, :]
                hn[b].append(_ln(v if tie is None else v + rep(zero_of(tie), LC)))
            def ffn1(b):
                u = (jnp.dot(jnp.concatenate(hn[b], axis=0).astype(bf16), w1_ref[...], preferred_element_type=f32)
                     + b1_ref[...].reshape(1, F).astype(f32))
                gl[b] = _gelu(u)
                return u
            def ffn2(b, tie=None):
                gg = gl[b]
                if tie is not None:
                    last = gg[:, F - 128:] + jnp.concatenate([zero_of(tie)] * 16, axis=0)
                    gg = jnp.concatenate([gg[:, :F - 128], last], axis=1)
                y = jnp.dot(gg.astype(bf16), w2_ref[...], preferred_element_type=f32) + b2_ref[...].reshape(1, D).astype(f32)
                o_ref[128 * b:128 * (b + 1), :] = (h_scr[128 * b:128 * (b + 1), :] + y).astype(o_ref.dtype)
                return y
            def ln_next(j, tie):
                st = BM + LC * j if first else pl.multiple_of(jnp.minimum(step + 1, NS - 1) * BM + LC * j, LC)
                y = _ln(x_scr[pl.ds(st, LC), :].astype(f32) + rep(zero_of(tie), LC))
                xn_scr[LC * j:LC * (j + 1), :] = y.astype(bf16)
                return functools.reduce(jnp.maximum, [y[8 * i:8 * i + 8, 512:640] for i in range(LC // 8)])

            NL = 128 // LC
            items = [(b, g) for b in range(NB) for g in range(8) if not (first and b == 1)]
            s_cur = qk(*items[0])
            for i, (b, g) in enumerate(items):
                s_nxt = qk(*items[i + 1]) if i + 1 < len(items) else None
                if first and i == W2_AT:
                    cp_w2.start()
                if b > 0:
                    if g == WO_AT:
                        wo(b - 1)
                    if WO_AT < g <= WO_AT + NL:
                        ln2(b - 1, s_nxt[1][-1])
                    if b > 1 and g == 0:
                        ffn2(b - 2)
                    if g == 7:
                        ffn1(b - 1)
                sm_pv(b, g, s_cur, s_nxt and s_nxt[1])
                s_cur = s_nxt
            if first:
                cp_wo.wait(); cp_x1.wait(); cp_w1.wait(); cp_b1.wait(); cp_b2.wait()
                wo(0); wo(1)
                for j in range(NL):
                    ln2(0)
                u = ffn1(0)
                for j in range(NL):
                    ln2(1, u[0:8, 256 * j:256 * j + 128])
                cp_w2.wait()
                cp_x2.start()
                u = ffn1(1)
                ffn2(0)
            else:
                wo(NB - 1)
                y = ffn2(NB - 2)
                for j in range(NL):
                    ln2(NB - 1, None if j == 0 else y[0:8, 128 * (j - 1):128 * j])
                u = ffn1(NB - 1)
            nl = BM // LC
            t = [ln_next(j, u[0:8, 128 * (j * 8 // nl):128 * (j * 8 // nl + 1)]) for j in range(nl)]
            ffn2(NB - 1, functools.reduce(jnp.maximum, t))
            if first:
                cp_x2.wait()

        pl.when(step == 0)(lambda: body(True))
        pl.when(step > 0)(lambda: body(False))

    def run(A_x, A_wqkv, A_wo, B_x, B_w1, B_b1, B_w2, B_b2):
        hbm = pl.BlockSpec(memory_space=pl.ANY)
        out = pl.pallas_call(
            kern,
            grid=(NS,),
            in_specs=[hbm] * 7,
            out_specs=pl.BlockSpec((BM, D), lambda i: (i, 0)),
            out_shape=jax.ShapeDtypeStruct((S, D), A_x.dtype),
            scratch_shapes=[pltpu.VMEM((F,), bf16), pltpu.VMEM((D,), bf16), pltpu.VMEM((S, D), bf16), pltpu.VMEM((D, 3 * D), bf16), pltpu.VMEM((D, D), bf16),
                            pltpu.VMEM((D, F), bf16), pltpu.VMEM((F, D), bf16), pltpu.VMEM((BM, D), bf16),
                            pltpu.VMEM((8, S, 128), bf16), pltpu.VMEM((S // 128, D, 128), bf16),
                            pltpu.VMEM((2, 192, 512), u32), pltpu.VMEM((2, 384, 512), f32), pltpu.VMEM((BM, D), f32), pltpu.SemaphoreType.DMA((11,))],
            compiler_params=pltpu.CompilerParams(dimension_semantics=("arbitrary",), vmem_limit_bytes=100 * 2**20, flags=FL or None),
            name="fused_blk",
        )(A_x.reshape(S, D), A_wqkv, A_wo, B_w1, B_b1, B_w2, B_b2)
        return out.reshape(1, S, D)
    return run


@jax.jit
def pallas_sequential_preLN__sliding_block__dense_activation_gelu__prompt_kernel(
    A_x, A_wqkv, A_wo, B_x, B_w1, B_b1, B_w2, B_b2,
):
    return make()(A_x, A_wqkv, A_wo, B_x, B_w1, B_b1, B_w2, B_b2)
```

```python
import functools

import jax
import jax.numpy as jnp
import numpy as np
from jax.experimental import pallas as pl
from jax.experimental.pallas import tpu as pltpu

S, D, DH, F = 2048, 640, 20, 1536
BM = 256
NS = S // BM
QSCALE = float(DH ** -0.5 * np.log2(np.e))
NEG = -1e30
GROUP_TILES = [(0, None), (0, 1), (1, None), (1, 2), (2, 3), (3, None), (3, 4), (4, None)]
QKV_CHUNKS = (0, 256, 640, 1024, 1408, 1920)
OUT_PIECES = ((0, 128), (128, 192), (192, 256))
f32, bf16, u32 = jnp.float32, jnp.bfloat16, jnp.uint32


def _ln(x):
    xc = x - jnp.mean(x, axis=-1, keepdims=True)
    return xc * jax.lax.rsqrt(jnp.mean(xc * xc, axis=-1, keepdims=True) + 1e-5)


def _gelu(h):
    c = float(np.sqrt(2 / np.pi))
    hh = 0.5 * h
    return hh + hh * jnp.tanh(h * (c + (c * 0.044715) * (h * h)))


def _dot(a, b):
    return jax.lax.dot_general(a, b, (((1,), (0,)), ((), ())), preferred_element_type=f32)


def _cat(xs, axis=0):
    return xs[0] if len(xs) == 1 else jnp.concatenate(xs, axis=axis)


def _iota(shape, dim):
    return jax.lax.broadcasted_iota(jnp.int32, shape, dim)


def _mm(a, w_ref, c0, c1, k0=0):
    rows = slice(k0, k0 + a.shape[1])
    nfull = (c1 - c0) // 128
    while (nfull * (a.shape[1] // 128)) % 4:
        nfull -= 1
    cm, q = c1 - 128 * nfull, a.shape[0] // 4
    outs = []
    if cm > c0:
        outs.append(_cat([_dot(a[q * i:q * (i + 1)], w_ref[rows, c0:cm]) for i in range(4)]))
    if nfull:
        outs.append(_dot(a, w_ref[rows, cm:c1]))
    return _cat(outs, 1)


def _pack16(v):
    n = v.shape[0] // 16
    lo = _cat([v[16 * m:16 * m + 8] for m in range(n)])
    hi = _cat([v[16 * m + 8:16 * m + 16] for m in range(n)])
    return pltpu.pack_elementwise([lo, hi], packed_dtype=bf16)


def _unshuffled(p):
    return (p & ~15) + ((p & 15) >> 1) + 8 * (p & 1)


def _after(x, tie):
    if tie is None:
        return x
    zero = jnp.minimum(jnp.maximum(tie, 0.0), 0.0)
    return x + _cat([_cat([zero] * (x.shape[1] // 128), 1)] * (x.shape[0] // 8))


def _kernel(x_hbm, wqkv_hbm, wo_hbm, w1_hbm, b1_hbm, w2_hbm, b2_hbm, o_hbm,
            x_scr, wqkv, wo, w1, b1, w2, b2, xn_scr, qt_scr, k_scr, vt_scr, qmask_scr, pmask_scr,
            s_scr, p_scr, h_scr, o_scr, in_sems, out_sems):
    step = pl.program_id(0)

    def copy_out(st, i):
        r0, r1 = OUT_PIECES[i]
        dst = r0 if isinstance(st, int) else pl.multiple_of(st * BM + r0, 64)
        return pltpu.make_async_copy(o_scr.at[st % 2, r0:r1], o_hbm.at[pl.ds(dst, r1 - r0)],
                                     out_sems.at[st % 2, i])

    def wait_out(st):
        for i in range(len(OUT_PIECES)):
            copy_out(st, i).wait()

    def body(first):
        st = 0 if first else step

        def rows_at(offset, per_step, size):
            start = st * per_step + offset
            return pl.ds(start if first else pl.multiple_of(start, 64), size)

        lane, sub = _iota((1, 128), 1), _iota((8, 128), 0)

        if first:
            chunks = list(zip(QKV_CHUNKS[:-1], QKV_CHUNKS[1:]))
            pairs = dict(x0=(x_hbm.at[0:BM], x_scr.at[0:BM]), x1=(x_hbm.at[BM:2 * BM], x_scr.at[BM:2 * BM]),
                         x2=(x_hbm.at[2 * BM:S], x_scr.at[2 * BM:S]), wo=(wo_hbm, wo), w1=(w1_hbm, w1),
                         b1=(b1_hbm, b1), w2=(w2_hbm, w2), b2=(b2_hbm, b2))
            pairs.update({j: (wqkv_hbm.at[:, c0:c1], wqkv.at[:, c0:c1]) for j, (c0, c1) in enumerate(chunks)})
            copies = {n: pltpu.make_async_copy(a, b, in_sems.at[i]) for i, (n, (a, b)) in enumerate(pairs.items())}

            def start(*names):
                for n in names:
                    copies[n].start()

            def wait(*names):
                for n in names:
                    copies[n].wait()

            queue = [(j,) for j in range(len(chunks))] + [("wo", "b1", "b2"), ("w1", "x1", "w2")]
            start("x0", 0)
            wait("x0")
            start(1)
            xn = _ln(x_scr[0:BM].astype(f32)).astype(bf16)
            parts = []
            for j, (c0, c1) in enumerate(chunks):
                wait(j)
                start(*queue[j + 2])
                parts.append(_mm(xn, wqkv, c0, c1))
            qkv = _cat(parts, 1)
        else:
            qkv = _mm(xn_scr[...], wqkv, 0, 3 * D)

        kt = [_pack16(qkv[:, D + 128 * t:D + 128 * (t + 1)]) for t in range(5)]
        for g, (t0, t1) in enumerate(GROUP_TILES):
            k_scr[g, rows_at(0, BM // 2, BM // 2), :] = (
                kt[t0] if t1 is None else jnp.where(lane >= 64, kt[t0], kt[t1]))
        q = qkv[:, 0:D] * QSCALE
        for b in range(2):
            for j in range(4):
                qj = q[128 * b + 32 * j:128 * b + 32 * j + 32]
                qt_scr[b, j] = pltpu.bitcast(_cat([qj] * 4).astype(bf16).T, u32)
            v = qkv[128 * b:128 * (b + 1), 2 * D:]
            for _ in range(2):
                v = pltpu.bitcast(_pack16(v), bf16).astype(f32)
            vt_scr[2 * st + b] = v.T

        if first:
            r, c = _iota((64, 128), 0), _iota((64, 128), 1)
            r = r + (r & 56)
            w = _iota((40, 128), 0)
            head = (w >= 10).astype(jnp.int32) + (w >= 20).astype(jnp.int32) + (w >= 30).astype(jnp.int32)
            for a in range(4):
                query = c ^ (32 * a)
                pmask_scr[a] = (jnp.where(_unshuffled(r) <= query, jnp.uint32(0xFFFF), jnp.uint32(0))
                                | jnp.where(_unshuffled(r + 8) <= query, jnp.uint32(0xFFFF0000), jnp.uint32(0)))
                qmask_scr[a] = jnp.where(head == ((_iota((40, 128), 1) >> 5) ^ a),
                                         jnp.uint32(0xFFFFFFFF), jnp.uint32(0))
        causal = _unshuffled(_iota((32, 128), 0)) <= (_iota((32, 128), 1) & 31)
        odd_quarter, upper_half = (lane & 32) != 0, (lane & 64) != 0

        def scores(b, g, r0):
            n = b + 1 if first else 3
            k0 = 8 * (3 - n)
            kw = k_scr[g, rows_at(0 if first else 64 * (b - 2), BM // 2, 64 * n), :]
            t = [None] * 4
            for j in (range(4) if n == 3 else (3, 2, 1, 0)):
                wq = qt_scr[b, j, 40 * g:40 * g + 40, :] & qmask_scr[j]
                pos = [(i - 5 * g) % 8 for i in range(8)]
                wq = _cat([wq[8 * i:8 * i + 8] if i < 5 else jnp.zeros((8, 128), u32) for i in pos])
                order = ([2 * j, 16 + 2 * j, 2 * j + 1, 17 + 2 * j] + list(range(8, 16))
                         + list(range(16, 16 + 2 * j)) + list(range(2 * j + 2, 8)))
                order = [k for k in order if k >= k0]
                s = _dot(pltpu.bitcast(_cat([kw[8 * (k - k0):8 * (k - k0) + 8] for k in order]), bf16),
                         pltpu.bitcast(wq, bf16))
                t[j] = {k: s[16 * i:16 * i + 16] for i, k in enumerate(order)}
            neg = jnp.full((16, 128), NEG, f32)

            def folded(j, k):
                if k >= 2 * j + 2:
                    return t[j].get(k, neg)
                if k < 2 * j:
                    return t[j][16 + k]
                return jnp.where(causal[16 * (k & 1):16 * (k & 1) + 16], t[j][16 + k], t[j].get(k, neg))

            xs = [_cat([folded(j, k) for k in range(16 if n > 1 else 8)]) for j in range(4)]
            ys = [jnp.where(odd_quarter, xs[j ^ 1], xs[j]) for j in range(4)]
            s = _cat([jnp.where(upper_half, ys[a ^ 2], ys[a]) for a in range(4)], 1)
            s_scr[g % 2, r0:r0 + s.shape[0], :] = s
            return jnp.max(s, axis=0, keepdims=True), [[v[0:8] for v in tj.values()] for tj in t]

        def qk(b, g):
            if first:
                m1, t = scores(1, g, 128)
                m0, _ = scores(0, g, 0)
                return [m0, m1, m1], [None, t[0][2], t[0][3]], None
            m, t = scores(b, g, 0)
            return [m, m], [None, t[3][1]], t[3][16]

        def softmax(g, maxes, ties):
            for j, m in enumerate(maxes):
                m = _after(jnp.broadcast_to(m, (8, 512)), ties and ties[j])
                e = jnp.exp2(s_scr[g % 2, 128 * j:128 * (j + 1), :] - _cat([m] * 16))
                p_scr[g % 2, 64 * j:64 * (j + 1), :] = _pack16(e)

        att_t = [[None] * (D // 8) for _ in range(2)]

        def pv(b, g):
            n = b + 1 if first else 3
            for a in range(4):
                h, cols = 4 * g + a, slice(128 * a, 128 * (a + 1))
                if first:
                    ps = [p_scr[g % 2, 64 * b:64 * (2 * b + 1), cols]]
                else:
                    pm = p_scr[g % 2, 0:64, cols]
                    new = pm & pmask_scr[a]
                    ps = [pm ^ new, new, p_scr[g % 2, 64:128, cols]]
                f0 = (DH * h) // 8
                vs = []
                for j in ((0,), (1, 0), (0, 2, 1))[n - 1]:
                    v = vt_scr[2 * st + b + 1 - n + j, 8 * f0:8 * f0 + 24, :]
                    vs.append(_cat([jnp.where(sub < 4, 1.0, v[0:8]), v[8:24]] if h % 2 else
                                   [v[0:16], jnp.where(sub >= 4, 1.0, v[16:24])]))
                o = _dot(_cat(vs, 1), pltpu.bitcast(_cat(ps), bf16))
                inv = 1.0 / jnp.broadcast_to(o[0:1] if h % 2 else o[20:21], (8, 128))
                for i in range(3):
                    val = o[8 * i:8 * (i + 1)] * inv
                    if a == 2:
                        val = pltpu.roll(val, 64, axis=1)
                    elif a % 2:
                        val = jnp.where(odd_quarter, pltpu.roll(val, 32 if a == 1 else 96, axis=1),
                                        pltpu.roll(val, 96 if a == 1 else 32, axis=1))
                    prev = att_t[b][f0 + i]
                    att_t[b][f0 + i] = val if prev is None else jnp.where(sub < 4, prev, val)

        hn, act = [[], []], [[], []]

        def proj(b, k0=0, k1=D):
            blk = slice(128 * b, 128 * (b + 1))
            att = _cat(att_t[b][k0 // 8:k1 // 8]).T.astype(bf16)
            base = x_scr[rows_at(128 * b, BM, 128), :].astype(f32) if k0 == 0 else h_scr[blk, :]
            h_scr[blk, :] = base + _mm(att, wo, 0, D, k0)

        def ln2(b, tie=None):
            r0 = 128 * b + 32 * len(hn[b])
            hn[b].append(_ln(_after(h_scr[r0:r0 + 32, :], tie)))

        def ffn1(b, c0=0, c1=F):
            u = _dot(_cat(hn[b]).astype(bf16), w1[:, c0:c1]) + b1[...].reshape(1, F).astype(f32)[:, c0:c1]
            act[b].append(_gelu(u))
            return u

        def ffn2(b, tie=None):
            for i, (r0, r1) in enumerate(OUT_PIECES):
                if r0 // 128 == b:
                    a = _cat(act[b], 1)[r0 - 128 * b:r1 - 128 * b]
                    if tie is not None:
                        a, tie = _cat([a[:, :F - 128], _after(a[:, F - 128:], tie)], 1), None
                    y = _dot(a.astype(bf16), w2[...]) + b2[...].reshape(1, D).astype(f32)
                    o_scr[st % 2, r0:r1, :] = (h_scr[r0:r1, :] + y).astype(o_scr.dtype)
                    copy_out(st, i).start()
            return y

        def ln1_next(j, tie):
            src = BM + 16 * j if first else pl.multiple_of(jnp.minimum(step + 1, NS - 1) * BM + 16 * j, 16)
            y = _ln(_after(x_scr[pl.ds(src, 16), :].astype(f32), tie))
            xn_scr[16 * j:16 * (j + 1), :] = y.astype(bf16)
            return jnp.maximum(y[0:8, D - 128:], y[8:16, D - 128:])

        tile = lambda y, c, r=0: y[r:r + 8, 128 * c:128 * (c + 1)]

        items = [(b, g) for b in range(1 if first else 2) for g in range(8)]
        cur = qk(*items[0])
        for i, (b, g) in enumerate(items):
            nxt = qk(*items[i + 1]) if i + 1 < len(items) else (None, None, None)
            ties = nxt[1]
            if first and g == 6:
                wait("wo")
            if first and g == 7:
                proj(0, 0, 384)
            if b == 1 and g == 1:
                proj(0)
            if b == 1 and 2 <= g < 6:
                ln2(0, nxt[2])
            if b == 1 and g == 7:
                u = ffn1(0, 0, 1024)
                ties = [tile(u, 0), tile(u, 2)]
            softmax(g, cur[0], ties)
            pv(b, g)
            if first:
                pv(1, g)
            cur = nxt

        if first:
            proj(1, 0, 384)
            proj(0, 384, D)
            proj(1, 384, D)
            for j in range(4):
                ln2(0)
            wait("x1", "w1", "b1", "b2")
            start("x2")
            u = ffn1(0)
            for j in range(4):
                ln2(1, tile(u, 2 * j))
            u = ffn1(1)
            wait("w2")
            ffn2(0)
        else:
            ffn1(0, 1024, F)
            proj(1)
            y = ffn2(0)
            for j in range(4):
                ln2(1, tile(y, j - 1) if j else None)
            u = ffn1(1)
        done = [ln1_next(j, tile(u, j // 2, 64 * (j % 2))) for j in range(BM // 16)]
        ffn2(1, functools.reduce(jnp.maximum, done))
        if first:
            wait("x2")

    pl.when(step == 0)(lambda: body(True))
    pl.when(step > 1)(lambda: wait_out(step - 2))
    pl.when(step > 0)(lambda: body(False))

    @pl.when(step == NS - 1)
    def _():
        wait_out(step - 1)
        wait_out(step)


@jax.jit
def pallas_sequential_preLN__sliding_block__dense_activation_gelu__prompt_kernel(
    A_x: jax.Array,
    A_wqkv: jax.Array,
    A_wo: jax.Array,
    B_x: jax.Array,
    B_w1: jax.Array,
    B_b1: jax.Array,
    B_w2: jax.Array,
    B_b2: jax.Array,
):
    hbm = pl.BlockSpec(memory_space=pl.ANY)
    vmem = pltpu.VMEM
    out = pl.pallas_call(
        _kernel,
        grid=(NS,),
        in_specs=[hbm] * 7,
        out_specs=hbm,
        out_shape=jax.ShapeDtypeStruct((S, D), A_x.dtype),
        scratch_shapes=[
            vmem((S, D), bf16),
            vmem((D, 3 * D), bf16), vmem((D, D), bf16),
            vmem((D, F), bf16), vmem((F,), bf16), vmem((F, D), bf16), vmem((D,), bf16),
            vmem((BM, D), bf16),
            vmem((2, 4, D // 2, 128), u32),
            vmem((8, S // 2, 128), u32),
            vmem((S // 128, D, 128), f32),
            vmem((4, 40, 128), u32), vmem((4, 64, 128), u32),
            vmem((2, 384, 512), f32),
            vmem((2, 192, 512), u32),
            vmem((BM, D), f32),
            vmem((2, BM, D), A_x.dtype),
            pltpu.SemaphoreType.DMA((8 + len(QKV_CHUNKS) - 1,)),
            pltpu.SemaphoreType.DMA((2, len(OUT_PIECES))),
        ],
        compiler_params=pltpu.CompilerParams(
            dimension_semantics=("arbitrary",), vmem_limit_bytes=64 * 2**20),
        name="fused_block",
    )(A_x.reshape(S, D), A_wqkv, A_wo, B_w1, B_b1, B_w2, B_b2)
    return out.reshape(1, S, D)
```

```python
import functools

import jax
import jax.numpy as jnp
import numpy as np
from jax.experimental import pallas as pl
from jax.experimental.pallas import tpu as pltpu

S, D, DH, F = 2048, 640, 20, 1536
BM = 256
NS = S // BM
QSCALE = float(DH ** -0.5 * np.log2(np.e))
NEG = -1e30
GROUP_TILES = [(0, None), (0, 1), (1, None), (1, 2), (2, 3), (3, None), (3, 4), (4, None)]
QKV_CHUNKS = (0, 256, 640, 1024, 1408, 1920)
OUT_PIECES = ((0, 128), (128, 192), (192, 256))
f32, bf16, u32 = jnp.float32, jnp.bfloat16, jnp.uint32


def _ln(x):
    xc = x - jnp.mean(x, axis=-1, keepdims=True)
    return xc * jax.lax.rsqrt(jnp.mean(xc * xc, axis=-1, keepdims=True) + 1e-5)


def _gelu(h):
    c = float(np.sqrt(2 / np.pi))
    hh = 0.5 * h
    return hh + hh * jnp.tanh(h * (c + (c * 0.044715) * (h * h)))


def _dot(a, b):
    return jax.lax.dot_general(a, b, (((1,), (0,)), ((), ())), preferred_element_type=f32)


def _cat(xs, axis=0):
    return xs[0] if len(xs) == 1 else jnp.concatenate(xs, axis=axis)


def _iota(shape, dim):
    return jax.lax.broadcasted_iota(jnp.int32, shape, dim)


def _mm(a, w_ref, c0, c1, k0=0):
    rows = slice(k0, k0 + a.shape[1])
    nfull = (c1 - c0) // 128
    while (nfull * (a.shape[1] // 128)) % 4:
        nfull -= 1
    cm, q = c1 - 128 * nfull, a.shape[0] // 4
    outs = []
    if cm > c0:
        outs.append(_cat([_dot(a[q * i:q * (i + 1)], w_ref[rows, c0:cm]) for i in range(4)]))
    if nfull:
        outs.append(_dot(a, w_ref[rows, cm:c1]))
    return _cat(outs, 1)


def _pack16(v, nearest=True):
    n = v.shape[0] // 16
    lo = _cat([v[16 * m:16 * m + 8] for m in range(n)])
    hi = _cat([v[16 * m + 8:16 * m + 16] for m in range(n)])
    if nearest:
        lo, hi = (pltpu.bitcast(x.astype(bf16).astype(f32), u32) for x in (lo, hi))
        return hi | (lo >> 16)
    return (pltpu.bitcast(hi, u32) & jnp.uint32(0xFFFF0000)) | (pltpu.bitcast(lo, u32) >> 16)


def _unshuffled(p):
    return (p & ~15) + ((p & 15) >> 1) + 8 * (p & 1)


def _after(x, tie):
    if tie is None:
        return x
    zero = jnp.minimum(jnp.maximum(tie, 0.0), 0.0)
    return x + _cat([_cat([zero] * (x.shape[1] // 128), 1)] * (x.shape[0] // 8))


def _kernel(x_hbm, wqkv_hbm, wo_hbm, w1_hbm, b1_hbm, w2_hbm, b2_hbm, o_hbm,
            x_scr, wqkv, wo, w1, b1, w2, b2, xn_scr, qt_scr, k_scr, vt_scr, qmask_scr, pmask_scr,
            s_scr, p_scr, h_scr, o_scr, in_sems, out_sems):
    step = pl.program_id(0)

    def copy_out(st, i):
        r0, r1 = OUT_PIECES[i]
        dst = r0 if isinstance(st, int) else pl.multiple_of(st * BM + r0, 64)
        return pltpu.make_async_copy(o_scr.at[st % 2, r0:r1], o_hbm.at[pl.ds(dst, r1 - r0)],
                                     out_sems.at[st % 2, i])

    def wait_out(st):
        for i in range(len(OUT_PIECES)):
            copy_out(st, i).wait()

    def body(first):
        st = 0 if first else step

        def rows_at(offset, per_step, size):
            start = st * per_step + offset
            return pl.ds(start if first else pl.multiple_of(start, 64), size)

        lane, sub = _iota((1, 128), 1), _iota((8, 128), 0)

        if first:
            chunks = list(zip(QKV_CHUNKS[:-1], QKV_CHUNKS[1:]))
            pairs = dict(x0=(x_hbm.at[0:BM], x_scr.at[0:BM]), x1=(x_hbm.at[BM:2 * BM], x_scr.at[BM:2 * BM]),
                         x2=(x_hbm.at[2 * BM:S], x_scr.at[2 * BM:S]), wo=(wo_hbm, wo), w1=(w1_hbm, w1),
                         b1=(b1_hbm, b1), w2=(w2_hbm, w2), b2=(b2_hbm, b2))
            pairs.update({j: (wqkv_hbm.at[:, c0:c1], wqkv.at[:, c0:c1]) for j, (c0, c1) in enumerate(chunks)})
            copies = {n: pltpu.make_async_copy(a, b, in_sems.at[i]) for i, (n, (a, b)) in enumerate(pairs.items())}

            def start(*names):
                for n in names:
                    copies[n].start()

            def wait(*names):
                for n in names:
                    copies[n].wait()

            queue = [(j,) for j in range(len(chunks))] + [("wo", "b1", "b2"), ("w1", "x1", "w2")]
            start("x0", 0)
            wait("x0")
            start(1)
            xn = _ln(x_scr[0:BM].astype(f32)).astype(bf16)
            parts = []
            for j, (c0, c1) in enumerate(chunks):
                wait(j)
                start(*queue[j + 2])
                parts.append(_mm(xn, wqkv, c0, c1))
            qkv = _cat(parts, 1)
        else:
            qkv = _mm(xn_scr[...], wqkv, 0, 3 * D)

        kt = [_pack16(qkv[:, D + 128 * t:D + 128 * (t + 1)]) for t in range(5)]
        for g, (t0, t1) in enumerate(GROUP_TILES):
            k_scr[g, rows_at(0, BM // 2, BM // 2), :] = (
                kt[t0] if t1 is None else jnp.where(lane >= 64, kt[t0], kt[t1]))
        q = qkv[:, 0:D] * QSCALE
        for b in range(2):
            for j in range(4):
                qj = q[128 * b + 32 * j:128 * b + 32 * j + 32]
                qt_scr[b, j] = pltpu.bitcast(_cat([qj] * 4).astype(bf16).T, u32)
            v = qkv[128 * b:128 * (b + 1), 2 * D:]
            for _ in range(2):
                v = pltpu.bitcast(_pack16(v), bf16).astype(f32)
            vt_scr[2 * st + b] = v.T

        if first:
            r, c = _iota((64, 128), 0), _iota((64, 128), 1)
            r = r + (r & 56)
            w = _iota((40, 128), 0)
            head = (w >= 10).astype(jnp.int32) + (w >= 20).astype(jnp.int32) + (w >= 30).astype(jnp.int32)
            for a in range(4):
                query = c ^ (32 * a)
                pmask_scr[a] = (jnp.where(_unshuffled(r) <= query, jnp.uint32(0xFFFF), jnp.uint32(0))
                                | jnp.where(_unshuffled(r + 8) <= query, jnp.uint32(0xFFFF0000), jnp.uint32(0)))
                qmask_scr[a] = jnp.where(head == ((_iota((40, 128), 1) >> 5) ^ a),
                                         jnp.uint32(0xFFFFFFFF), jnp.uint32(0))
        causal = _unshuffled(_iota((32, 128), 0)) <= (_iota((32, 128), 1) & 31)
        odd_quarter, upper_half = (lane & 32) != 0, (lane & 64) != 0

        def scores(b, g, r0):
            n = b + 1 if first else 3
            k0 = 8 * (3 - n)
            kw = k_scr[g, rows_at(0 if first else 64 * (b - 2), BM // 2, 64 * n), :]
            t = [None] * 4
            for j in (range(4) if n == 3 else (3, 2, 1, 0)):
                wq = qt_scr[b, j, 40 * g:40 * g + 40, :] & qmask_scr[j]
                pos = [(i - 5 * g) % 8 for i in range(8)]
                wq = _cat([wq[8 * i:8 * i + 8] if i < 5 else jnp.zeros((8, 128), u32) for i in pos])
                order = ([2 * j, 16 + 2 * j, 2 * j + 1, 17 + 2 * j] + list(range(8, 16))
                         + list(range(16, 16 + 2 * j)) + list(range(2 * j + 2, 8)))
                order = [k for k in order if k >= k0]
                s = _dot(pltpu.bitcast(_cat([kw[8 * (k - k0):8 * (k - k0) + 8] for k in order]), bf16),
                         pltpu.bitcast(wq, bf16))
                t[j] = {k: s[16 * i:16 * i + 16] for i, k in enumerate(order)}
            neg = jnp.full((16, 128), NEG, f32)

            def folded(j, k):
                if k >= 2 * j + 2:
                    return t[j].get(k, neg)
                if k < 2 * j:
                    return t[j][16 + k]
                return jnp.where(causal[16 * (k & 1):16 * (k & 1) + 16], t[j][16 + k], t[j].get(k, neg))

            xs = [_cat([folded(j, k) for k in range(16 if n > 1 else 8)]) for j in range(4)]
            ys = [jnp.where(odd_quarter, xs[j ^ 1], xs[j]) for j in range(4)]
            s = _cat([jnp.where(upper_half, ys[a ^ 2], ys[a]) for a in range(4)], 1)
            s_scr[g % 2, r0:r0 + s.shape[0], :] = s
            return jnp.max(s, axis=0, keepdims=True), [[v[0:8] for v in tj.values()] for tj in t]

        def qk(b, g):
            if first:
                m1, t = scores(1, g, 128)
                m0, _ = scores(0, g, 0)
                return [m0, m1, m1], [None, t[0][2], t[0][3]], None
            m, t = scores(b, g, 0)
            return [m, m], [None, t[3][2]], t[3][16]

        def softmax(g, maxes, ties):
            for j, m in enumerate(maxes):
                m = _after(jnp.broadcast_to(m, (8, 512)), ties and ties[j])
                e = jnp.exp2(s_scr[g % 2, 128 * j:128 * (j + 1), :] - _cat([m] * 16))
                p_scr[g % 2, 64 * j:64 * (j + 1), :] = _pack16(e, nearest=False)

        att_t = [[None] * (D // 8) for _ in range(2)]

        def pv(b, g):
            n = b + 1 if first else 3
            for a in range(4):
                h, cols = 4 * g + a, slice(128 * a, 128 * (a + 1))
                if first:
                    ps = [p_scr[g % 2, 64 * b:64 * (2 * b + 1), cols]]
                else:
                    pm = p_scr[g % 2, 0:64, cols]
                    new = pm & pmask_scr[a]
                    ps = [pm ^ new, new, p_scr[g % 2, 64:128, cols]]
                f0 = (DH * h) // 8
                vs = []
                for j in ((0,), (1, 0), (0, 2, 1))[n - 1]:
                    v = vt_scr[2 * st + b + 1 - n + j, 8 * f0:8 * f0 + 24, :]
                    vs.append(_cat([jnp.where(sub < 4, 1.0, v[0:8]), v[8:24]] if h % 2 else
                                   [v[0:16], jnp.where(sub >= 4, 1.0, v[16:24])]))
                o = _dot(_cat(vs, 1), pltpu.bitcast(_cat(ps), bf16))
                inv = 1.0 / jnp.broadcast_to(o[0:1] if h % 2 else o[20:21], (8, 128))
                for i in range(3):
                    val = o[8 * i:8 * (i + 1)] * inv
                    if a == 2:
                        val = pltpu.roll(val, 64, axis=1)
                    elif a % 2:
                        val = jnp.where(odd_quarter, pltpu.roll(val, 32 if a == 1 else 96, axis=1),
                                        pltpu.roll(val, 96 if a == 1 else 32, axis=1))
                    prev = att_t[b][f0 + i]
                    att_t[b][f0 + i] = val if prev is None else jnp.where(sub < 4, prev, val)

        hn, act = [[], []], [[], []]

        def proj(b, k0=0, k1=D):
            blk = slice(128 * b, 128 * (b + 1))
            att = _cat(att_t[b][k0 // 8:k1 // 8]).T.astype(bf16)
            base = x_scr[rows_at(128 * b, BM, 128), :].astype(f32) if k0 == 0 else h_scr[blk, :]
            h_scr[blk, :] = base + _mm(att, wo, 0, D, k0)

        def ln2(b, tie=None):
            r0 = 128 * b + 32 * len(hn[b])
            hn[b].append(_ln(_after(h_scr[r0:r0 + 32, :], tie)))

        def ffn1(b, c0=0, c1=F):
            u = _dot(_cat(hn[b]).astype(bf16), w1[:, c0:c1]) + b1[...].reshape(1, F).astype(f32)[:, c0:c1]
            act[b].append(_gelu(u))
            return u

        def ffn2(b, tie=None):
            for i, (r0, r1) in enumerate(OUT_PIECES):
                if r0 // 128 == b:
                    a = _cat(act[b], 1)[r0 - 128 * b:r1 - 128 * b]
                    if tie is not None:
                        a, tie = _cat([a[:, :F - 128], _after(a[:, F - 128:], tie)], 1), None
                    y = _dot(a.astype(bf16), w2[...]) + b2[...].reshape(1, D).astype(f32)
                    o_scr[st % 2, r0:r1, :] = (h_scr[r0:r1, :] + y).astype(o_scr.dtype)
                    copy_out(st, i).start()
            return y

        def ln1_next(j, tie):
            src = BM + 16 * j if first else pl.multiple_of(jnp.minimum(step + 1, NS - 1) * BM + 16 * j, 16)
            y = _ln(_after(x_scr[pl.ds(src, 16), :].astype(f32), tie))
            xn_scr[16 * j:16 * (j + 1), :] = y.astype(bf16)
            return jnp.maximum(y[0:8, D - 128:], y[8:16, D - 128:])

        tile = lambda y, c, r=0: y[r:r + 8, 128 * c:128 * (c + 1)]

        items = [(b, g) for b in range(1 if first else 2) for g in range(8)]
        cur = qk(*items[0])
        for i, (b, g) in enumerate(items):
            nxt = qk(*items[i + 1]) if i + 1 < len(items) else (None, None, None)
            ties = nxt[1]
            if first and g == 6:
                wait("wo")
            if first and g == 7:
                proj(0, 0, 384)
            if b == 1 and g == 1:
                proj(0)
            if b == 1 and 2 <= g < 6:
                ln2(0, nxt[2])
            if b == 1 and g == 7:
                u = ffn1(0, 0, 1024)
                ties = [tile(u, 0), tile(u, 2)]
            softmax(g, cur[0], ties)
            pv(b, g)
            if first:
                pv(1, g)
            cur = nxt

        if first:
            proj(1, 0, 384)
            proj(0, 384, D)
            proj(1, 384, D)
            for j in range(4):
                ln2(0)
            wait("x1", "w1", "b1", "b2")
            start("x2")
            u = ffn1(0)
            for j in range(4):
                ln2(1, tile(u, 2 * j))
            u = ffn1(1)
            wait("w2")
            ffn2(0)
        else:
            ffn1(0, 1024, F)
            proj(1)
            y = ffn2(0)
            for j in range(4):
                ln2(1, tile(y, j - 1) if j else None)
            u = ffn1(1)
        done = [ln1_next(j, tile(u, j // 2, 64 * (j % 2))) for j in range(BM // 16)]
        ffn2(1, functools.reduce(jnp.maximum, done))
        if first:
            wait("x2")

    pl.when(step == 0)(lambda: body(True))
    pl.when(step > 1)(lambda: wait_out(step - 2))
    pl.when(step > 0)(lambda: body(False))

    @pl.when(step == NS - 1)
    def _():
        wait_out(step - 1)
        wait_out(step)


@jax.jit
def pallas_sequential_preLN__sliding_block__dense_activation_gelu__prompt_kernel(
    A_x: jax.Array,
    A_wqkv: jax.Array,
    A_wo: jax.Array,
    B_x: jax.Array,
    B_w1: jax.Array,
    B_b1: jax.Array,
    B_w2: jax.Array,
    B_b2: jax.Array,
):
    hbm = pl.BlockSpec(memory_space=pl.ANY)
    vmem = pltpu.VMEM
    out = pl.pallas_call(
        _kernel,
        grid=(NS,),
        in_specs=[hbm] * 7,
        out_specs=hbm,
        out_shape=jax.ShapeDtypeStruct((S, D), A_x.dtype),
        scratch_shapes=[
            vmem((S, D), bf16),
            vmem((D, 3 * D), bf16), vmem((D, D), bf16),
            vmem((D, F), bf16), vmem((F,), bf16), vmem((F, D), bf16), vmem((D,), bf16),
            vmem((BM, D), bf16),
            vmem((2, 4, D // 2, 128), u32),
            vmem((8, S // 2, 128), u32),
            vmem((S // 128, D, 128), f32),
            vmem((4, 40, 128), u32), vmem((4, 64, 128), u32),
            vmem((2, 384, 512), f32),
            vmem((2, 192, 512), u32),
            vmem((BM, D), f32),
            vmem((2, BM, D), A_x.dtype),
            pltpu.SemaphoreType.DMA((8 + len(QKV_CHUNKS) - 1,)),
            pltpu.SemaphoreType.DMA((2, len(OUT_PIECES))),
        ],
        compiler_params=pltpu.CompilerParams(
            dimension_semantics=("arbitrary",), vmem_limit_bytes=64 * 2**20),
        name="fused_block",
    )(A_x.reshape(S, D), A_wqkv, A_wo, B_w1, B_b1, B_w2, B_b2)
    return out.reshape(1, S, D)
```
